```python
import os as _os
_os.environ.setdefault('JAX_PLATFORMS', 'cpu')
import jax
import jax.numpy as jnp

def _softmax(x, axis=-1):
    return jax.nn.softmax(x, axis=axis)

def _gelu(x):
    return jax.nn.gelu(x, approximate=True)

def _silu(x):
    return jax.nn.silu(x)

def _sigmoid(x):
    return jax.nn.sigmoid(x)

def _layernorm(x, axis=-1, eps=1e-05):
    m = jnp.mean(x, axis=axis, keepdims=True)
    v = jnp.var(x, axis=axis, keepdims=True)
    return (x - m) / jnp.sqrt(v + eps)

def _scatter_add(tgt, idx, src, axis=0):
    return tgt.at[idx].add(src)

def _segment_sum(src, seg, n):
    return jax.ops.segment_sum(src, seg, n)

class _Rng:

    def __init__(self, key):
        self._k = key

    def _next(self):
        self._k, sub = jax.random.split(self._k)
        return sub

    def normal(self, shape):
        return jax.random.normal(self._next(), shape, dtype=jnp.bfloat16)

    def randint(self, lo, hi, shape):
        return jax.random.randint(self._next(), shape, lo, hi, dtype=jnp.int32)

    def uniform(self, shape, lo=0.0, hi=1.0):
        return jax.random.uniform(self._next(), shape, jnp.bfloat16, lo, hi)

    def permutation(self, n):
        return jax.random.permutation(self._next(), n)
kernel_name = 'adaLN_cond__memory_aug_recurrent_mem_tr__moe_arch_mod__prompt'

def setup_inputs():
    _rng = _Rng(jax.random.key(int.from_bytes(__import__("os").urandom(4), "little")))
    _w = lambda a: (lambda t: t.astype(jnp.bfloat16) if jnp.issubdtype(t.dtype, jnp.floating) else t)(jnp.asarray(a))

    def _A_setup():
        B, S, Dm = (1, 2048, 448)
        H, Dh = (16, 256)
        M, seg = (8, 32)
        seg = min(seg, S)
        S = S // seg * seg
        return {'x': _w((lambda *s: _rng.normal(s) * 0.05)(B, S, Dm)), 'mem0': _w((lambda *s: _rng.normal(s) * 0.4)(B, M, Dm)), 'Wq': _w((lambda *s: _rng.normal(s) * 1.6)(Dm, H, Dh) * Dm ** (-0.5)), 'Wk': _w((lambda *s: _rng.normal(s) * 1.6)(Dm, H, Dh) * Dm ** (-0.5)), 'Wv': _w((lambda *s: _rng.normal(s) * 0.4)(Dm, H, Dh) * Dm ** (-0.5)), 'Wo': _w((lambda *s: _rng.normal(s) * 0.4)(H, Dh, Dm) * (H * Dh) ** (-0.5)), 'seg_len': seg}
    _A_in = _A_setup()

    def _B_setup():
        B, S, D, F, C = (1, 2048, 448, 1792, 1)
        return {'x': _w((lambda *s: _rng.normal(s) * 0.05)(B, S, D)), 'w_r': _w((lambda *s: _rng.normal(s) * 0.05)(D)), 'w_gate': _w((lambda *s: _rng.normal(s) * 0.05)(D, F)), 'w_up': _w((lambda *s: _rng.normal(s) * 0.05)(D, F)), 'w_down': _w((lambda *s: _rng.normal(s) * 0.05)(F, D))}
    _B_in = _B_setup()
    return {'A_x': _A_in['x'], 'A_mem0': _A_in['mem0'], 'A_Wq': _A_in['Wq'], 'A_Wk': _A_in['Wk'], 'A_Wv': _A_in['Wv'], 'A_Wo': _A_in['Wo'], 'A_seg_len': _A_in['seg_len'], 'B_x': _B_in['x'], 'B_w_r': _B_in['w_r'], 'B_w_gate': _B_in['w_gate'], 'B_w_up': _B_in['w_up'], 'B_w_down': _B_in['w_down'], 'c': _w((lambda *s: _rng.normal(s) * 0.05)(1, 448) * 8.0), 'w_mod': _w((lambda *s: _rng.normal(s) * 0.05)(448, 6 * 448) * 448 ** (-0.5) * 8.0)}

def reference(A_x, A_mem0, A_Wq, A_Wk, A_Wv, A_Wo, A_seg_len, B_x, B_w_r, B_w_gate, B_w_up, B_w_down, c, w_mod):

    def _A_ref(x, mem0, Wq, Wk, Wv, Wo, seg_len):
        B, S, Dm = x.shape
        H, Dh = (Wq.shape[1], Wq.shape[2])
        M = mem0.shape[1]
        scale = Dh ** (-0.5)
        n_seg = S // seg_len
        L = M + seg_len
        idx = jnp.arange(L)
        mask = (idx[:, None] < M) | (idx[:, None] >= idx[None, :])
        mem = mem0
        outs = []
        for s in range(n_seg):
            xs = x[:, s * seg_len:(s + 1) * seg_len, :].copy()
            h = jnp.concatenate([mem, xs], axis=1)
            q = jnp.einsum('btd,dhe->bhte', h, Wq)
            k = jnp.einsum('btd,dhe->bhte', h, Wk)
            v = jnp.einsum('btd,dhe->bhte', h, Wv)
            scores = jnp.einsum('bhqe,bhke->bhqk', q, k) * scale
            scores = jnp.where(mask[None, None], scores, -1000000000.0)
            p = _softmax(scores, axis=-1)
            o = jnp.einsum('bhqk,bhke->bhqe', p, v)
            o = jnp.einsum('bhte,hed->btd', o, Wo)
            mem = o[:, :M, :].copy()
            outs.append(o[:, M:, :])
        return jnp.concatenate(outs, axis=1)

    def _B_ref(x, w_r, w_gate, w_up, w_down):
        B, S, D = x.shape
        C = 1
        r = x @ w_r
        idx = jnp.argsort(-r, axis=-1)[:, :C]
        idx_e = jnp.repeat(idx.reshape(B, C, 1), D, axis=2)
        x_sel = jnp.take_along_axis(x, idx_e, axis=1)
        g = _silu(x_sel @ w_gate)
        u = x_sel @ w_up
        y = g * u @ w_down
        r_sel = _sigmoid(jnp.take_along_axis(r, idx, axis=1))
        y = y * r_sel.reshape(B, C, 1)
        b_off = (jnp.arange(B) * S).reshape(B, 1)
        flat_idx = (idx + b_off).reshape(B * C)
        zero = (x * 0.0).reshape(B * S, D)
        upd = _scatter_add(zero, flat_idx, y.reshape(B * C, D), axis=0)
        return x + upd.reshape(B, S, D)
    x = A_x
    mod = (_silu(c) @ w_mod).reshape(c.shape[0], 6, 1, -1)
    sa, ca, ga, sb, cb, gb = (mod[:, 0].copy(), mod[:, 1].copy(), mod[:, 2].copy(), mod[:, 3].copy(), mod[:, 4].copy(), mod[:, 5].copy())
    h = _layernorm(x, axis=-1) * (1 + ca) + sa
    x = x + ga * _A_ref(h, A_mem0, A_Wq, A_Wk, A_Wv, A_Wo, A_seg_len)
    h = _layernorm(x, axis=-1) * (1 + cb) + sb
    x = x + gb * _B_ref(h, B_w_r, B_w_gate, B_w_up, B_w_down)
    return x
```

```python
import functools

import jax
import jax.numpy as jnp
import jax.experimental.pallas as pl
import jax.experimental.pallas.tpu as pltpu

f32 = jnp.float32
bf16 = jnp.bfloat16
u32 = jnp.uint32

S = 2048
D = 448
H = 16
DH = 256
M = 8
SEG = 32
NSEG = S // SEG
L = M + SEG
F = 1792
DP = 512
EPS = 1e-5
NEG = -1000000000.0

CH = 112
NCH = D // CH
UNROLL = 2
X1 = 2
X2 = 2
NT = (((1,), (1,)), ((), ()))


def _dup_tail(v):
    return jnp.concatenate([v, v[:, 384:448]], axis=1)


def _rb(v):
    return v.astype(bf16).astype(f32)


def _ln(x):
    mu = jnp.mean(x, axis=-1, keepdims=True)
    xc = x - mu
    var = jnp.mean(xc * xc, axis=-1, keepdims=True)
    return xc * jax.lax.rsqrt(var + EPS)


def _kernel(x_hbm, mem0_ref, wq_hbm, wk_hbm, wv_hbm, wo_hbm, wr_ref, wg_hbm, wu_hbm, wd_hbm,
            c_ref, wmod_hbm, out_ref,
            rawq, rawk, rawv, q_s, wo_v, w_s, scr_a, scr_b, x_v, h_all, att, x1_all, h2_all,
            wg_v, wu_v, wd_v, wmod_v, sems):
    def chunk_copies(src, dst, k, i):
        r0 = pl.multiple_of(i * (CH * H), CH * H)
        return [pltpu.make_async_copy(src.at[pl.ds(r0, CH * H), pl.ds(j * 128, 128)],
                                      dst.at[j, pl.ds(r0, CH * H), :],
                                      sems.at[k + 2 * i + j]) for j in range(2)]

    cp_o = pltpu.make_async_copy(wo_hbm, wo_v, sems.at[24])
    cp_x = pltpu.make_async_copy(x_hbm, x_v, sems.at[25])
    cp_m = pltpu.make_async_copy(wmod_hbm, wmod_v, sems.at[26])
    cp_g = pltpu.make_async_copy(wg_hbm, wg_v, sems.at[27])
    cp_u = pltpu.make_async_copy(wu_hbm, wu_v, sems.at[28])
    cp_d = pltpu.make_async_copy(wd_hbm, wd_v, sems.at[29])
    for i in range(NCH):
        for cp in chunk_copies(wq_hbm, rawq, 0, i):
            cp.start()
    for i in range(NCH):
        for cp in chunk_copies(wk_hbm, rawk, 8, i):
            cp.start()
    cp_o.start()
    for i in range(NCH):
        for cp in chunk_copies(wv_hbm, rawv, 16, i):
            cp.start()
    cp_x.start()
    cp_m.start()

    def head_pair(raw, i, p):
        r0 = pl.multiple_of(i * (CH * 8), CH * 8)
        r32 = raw.bitcast(u32)
        vs = [r32.at[j, pl.ds(r0, CH * 8), :][pl.ds(p, CH, stride=8), :] for j in range(2)]
        return [jnp.concatenate(
            [pltpu.unpack_elementwise(v, index=t, packed_dtype=bf16, unpacked_dtype=f32) for v in vs],
            axis=1) for t in range(2)]

    def store_pair(part, i, p, lo, hi):
        base = part * 56
        rows = pl.ds(pl.multiple_of(i * (CH // 2), 8), CH // 2)
        for t, a in enumerate((lo, hi)):
            for c in range(3):
                w_s[base + 8 + 16 * c + 2 * p + t, rows, :] = pltpu.bitcast(
                    a[:, c * 128:(c + 1) * 128].astype(bf16), u32)
        tl = jnp.concatenate([lo[:, 384:448], hi[:, 384:448]], axis=1)
        w_s[base + p, rows, :] = pltpu.bitcast(tl.astype(bf16), u32)

    def relayout_q(i, carry):
        for cp in chunk_copies(wq_hbm, rawq, 0, i):
            cp.wait()
        rows = pl.ds(pl.multiple_of(i * CH, 16), CH)
        for p in range(8):
            qs = head_pair(rawq, i, p)
            for t in range(2):
                q_s[2 * p + t, rows, :] = qs[t].astype(bf16)
        return carry

    jax.lax.fori_loop(0, NCH, relayout_q, 0)

    def fold_a(i, carry):
        for cp in chunk_copies(wk_hbm, rawk, 8, i):
            cp.wait()
        for p in range(8):
            ks = head_pair(rawk, i, p)
            a = [jax.lax.dot_general(ks[t], q_s[2 * p + t], NT, preferred_element_type=f32)
                 * (DH ** -0.5) for t in range(2)]
            store_pair(0, i, p, a[0], a[1])
        return carry

    jax.lax.fori_loop(0, NCH, fold_a, 0)

    cp_o.wait()

    def fold_b(i, carry):
        for cp in chunk_copies(wv_hbm, rawv, 16, i):
            cp.wait()
        for p in range(8):
            vs = head_pair(rawv, i, p)
            b = [jnp.dot(vs[t], wo_v[2 * p + t], preferred_element_type=f32) for t in range(2)]
            store_pair(1, i, p, b[0], b[1])
        return carry

    jax.lax.fori_loop(0, NCH, fold_b, 0)

    cp_x.wait()
    cp_m.wait()
    for cp in (cp_g, cp_u, cp_d):
        cp.start()

    cc = c_ref[...].astype(f32)
    sc = _rb(cc * jax.nn.sigmoid(cc))
    mod = jnp.dot(jnp.broadcast_to(sc, (8, D)), wmod_v[...], preferred_element_type=f32)[0:1]
    sa, ca, ga, sb, cb, gb = [mod[:, k * D:(k + 1) * D] for k in range(6)]
    ca1 = 1.0 + ca
    cb1 = 1.0 + cb
    wr = wr_ref[...].astype(f32).reshape(1, D)

    def seg_rows(s):
        return pl.ds(pl.multiple_of(s * SEG, SEG), SEG)

    def ln1(s):
        x = x_v[seg_rows(s), :].astype(f32)
        h_all[seg_rows(s), :] = _dup_tail(_rb(_ln(x) * ca1 + sa))

    row_iota = jax.lax.broadcasted_iota(jnp.int32, (SEG, 1), 0)

    def finish(s, valid, best, bidx):
        x = x_v[seg_rows(s), :].astype(f32)
        x1 = x + ga * att[:, :D]
        h2 = _ln(x1) * cb1 + sb
        x1_all[seg_rows(s), :] = x1
        h2_all[seg_rows(s), :] = h2
        out_ref[seg_rows(s), :] = (x1 + gb * h2).astype(out_ref.dtype)
        r = jnp.sum(h2 * wr, axis=-1, keepdims=True)
        better = jnp.logical_and(r > best, valid)
        return jnp.where(better, r, best), jnp.where(better, row_iota + s * SEG, bidx)

    qi = jax.lax.broadcasted_iota(jnp.int32, (L, 128), 0)
    ki = jax.lax.broadcasted_iota(jnp.int32, (L, 128), 1) // H

    def unit(lhs, row0, scr, part, u):
        n = lhs.shape[0]
        t0 = part * 56 + 2 * u
        w = jnp.concatenate([pltpu.bitcast(w_s[t0 + j], bf16) for j in range(2)], axis=1)
        y = jnp.dot(lhs, w, preferred_element_type=f32)
        if u >= 4:
            c, p = (u - 4) // 8, (u - 4) % 8
            pk = pltpu.pack_elementwise([y[:, :128], y[:, 128:]], packed_dtype=bf16)
            scr[c, pl.ds(row0 * 8 + p, n, stride=8), :] = pk
        else:
            lane = jax.lax.broadcasted_iota(jnp.int32, (n, 128), 1)
            for j in range(2):
                t = y[:, j * 128:(j + 1) * 128]
                pk = pltpu.pack_elementwise(
                    [jnp.where(lane < 64, t, 0.0), jnp.where(lane >= 64, t, 0.0)], packed_dtype=bf16)
                scr[3, pl.ds(row0 * 8 + 2 * u + j, n, stride=8), :] = pk

    X = X1 + X2
    ln1(0)
    att[...] = jnp.zeros(att.shape, f32)
    hx0 = h_all[seg_rows(0), :D]
    for u in range(X):
        unit(hx0, M, scr_a, 0, u)

    def step(s, carry):
        mem, best, bidx = carry
        sn = jnp.minimum(s + 1, NSEG - 1)
        best, bidx = finish(jnp.maximum(s - 1, 0), s > 0, best, bidx)
        ln1(sn)
        h40 = jnp.concatenate([mem, h_all[seg_rows(s), :]], axis=0)
        h40a = h40[:, :D]
        k = 0
        for i, u in enumerate(range(X, 28)):
            unit(h40a, 0, scr_a, 0, u)
            if i % 3 == 2 and k < X:
                unit(h40a[:M], 0, scr_a, 0, k)
                k += 1
        st = []

        def s_tile(t):
            kst = jnp.concatenate(
                [pltpu.bitcast(scr_a[c, t * 64:(t + 1) * 64, :], bf16) for c in range(4)], axis=1)
            sc_ = jax.lax.dot_general(h40, kst, NT, preferred_element_type=f32)
            mask = jnp.logical_or(qi < M, qi >= ki + 8 * t)
            st.append(jnp.where(mask, sc_, NEG))

        for u in range(12):
            unit(h40a, 0, scr_b, 1, u)
            if u >= 2 and u % 2 == 0:
                s_tile(len(st))
        m = st[0]
        for t in range(1, 5):
            m = jnp.maximum(m, st[t])
        for sh in (16, 32, 64):
            m = jnp.maximum(m, pltpu.roll(m, sh, 1))
        e = [jnp.exp(st[t] - m) for t in range(5)]
        l = e[0] + e[1] + e[2] + e[3] + e[4]
        for sh in (16, 32, 64):
            l = l + pltpu.roll(l, sh, 1)
        r = 1.0 / l
        p = jnp.concatenate([_rb(v * r) for v in e], axis=1)

        def pz(c):
            return jnp.dot(p, pltpu.bitcast(scr_b[c], bf16), preferred_element_type=f32)

        for u in range(12, 24):
            unit(h40a, 0, scr_b, 1, u)
        tl = pz(3)
        o0 = pz(0)
        for u in range(24, 28):
            unit(h40a, 0, scr_b, 1, u)
        o1 = pz(1)
        hn = h_all[seg_rows(sn), :D]
        for u in range(X1):
            unit(hn, M, scr_a, 0, u)
        o2 = pz(2)
        for u in range(X1, X):
            unit(hn, M, scr_a, 0, u)
        tl = tl + pltpu.roll(tl, 64, 1)
        o = jnp.concatenate([o0, o1, o2, tl], axis=1)
        att[...] = o[M:]
        return _rb(o[:M]), best, bidx

    mem0 = _dup_tail(mem0_ref[...].astype(f32))
    best0 = jnp.full((SEG, 1), -jnp.inf, f32)
    bidx0 = jnp.zeros((SEG, 1), jnp.int32)
    _, best, bidx = jax.lax.fori_loop(0, NSEG, step, (mem0, best0, bidx0), unroll=UNROLL)
    best, bidx = finish(NSEG - 1, True, best, bidx)

    rmax = jnp.max(best, axis=0, keepdims=True)
    idx = jnp.min(jnp.where(best == rmax, bidx, S))
    idx = jnp.clip(idx, 0, S - 1)
    base = pl.multiple_of((idx // 16) * 16, 16)
    for cp in (cp_g, cp_u, cp_d):
        cp.wait()
    xs = _rb(jnp.broadcast_to(h2_all[pl.ds(idx, 1), :], (8, D)))
    g = jnp.dot(xs, wg_v[...], preferred_element_type=f32)
    u = jnp.dot(xs, wu_v[...], preferred_element_type=f32)
    a = _rb(g * jax.nn.sigmoid(g) * u)
    y = jnp.dot(a, wd_v[...], preferred_element_type=f32)[0:1] * jax.nn.sigmoid(rmax)
    sel = jax.lax.broadcasted_iota(jnp.int32, (16, 1), 0) == (idx - base)
    h2 = h2_all[pl.ds(base, 16), :]
    h2 = h2 + jnp.where(sel, y, 0.0)
    out_ref[pl.ds(base, 16), :] = (x1_all[pl.ds(base, 16), :] + gb * h2).astype(out_ref.dtype)


@functools.partial(jax.jit, static_argnames=("A_seg_len",))
def pallas_adaLN_cond__memory_aug_recurrent_mem_tr__moe_arch_mod__prompt_kernel(
    A_x, A_mem0, A_Wq, A_Wk, A_Wv, A_Wo, A_seg_len, B_x, B_w_r, B_w_gate, B_w_up, B_w_down,
    c, w_mod,
):
    del B_x
    assert int(A_seg_len) == SEG and A_x.shape == (1, S, D)
    any_spec = pl.BlockSpec(memory_space=pl.ANY)
    vmem_spec = pl.BlockSpec(memory_space=pltpu.VMEM)
    out = pl.pallas_call(
        _kernel,
        out_shape=jax.ShapeDtypeStruct((S, D), A_x.dtype),
        in_specs=[any_spec, vmem_spec, any_spec, any_spec, any_spec, any_spec, vmem_spec,
                  any_spec, any_spec, any_spec, vmem_spec, any_spec],
        out_specs=vmem_spec,
        scratch_shapes=[
            pltpu.VMEM((2, D * H, 128), bf16),
            pltpu.VMEM((2, D * H, 128), bf16),
            pltpu.VMEM((2, D * H, 128), bf16),
            pltpu.VMEM((H, D, DH), bf16),
            pltpu.VMEM((H, DH, D), bf16),
            pltpu.VMEM((112, D // 2, 128), u32),
            pltpu.VMEM((4, L * 8, 128), u32),
            pltpu.VMEM((4, L * 8, 128), u32),
            pltpu.VMEM((S, D), bf16),
            pltpu.VMEM((S, DP), f32),
            pltpu.VMEM((SEG, DP), f32),
            pltpu.VMEM((S, D), f32),
            pltpu.VMEM((S, D), f32),
            pltpu.VMEM((D, F), bf16),
            pltpu.VMEM((D, F), bf16),
            pltpu.VMEM((F, D), bf16),
            pltpu.VMEM((D, 6 * D), bf16),
            pltpu.SemaphoreType.DMA((30,)),
        ],
        compiler_params=pltpu.CompilerParams(vmem_limit_bytes=100 * 1024 * 1024),
    )(
        A_x.reshape(S, D), A_mem0.reshape(M, D),
        A_Wq.reshape(D * H, DH), A_Wk.reshape(D * H, DH), A_Wv.reshape(D * H, DH), A_Wo,
        B_w_r, B_w_gate, B_w_up, B_w_down, c, w_mod,
    )
    return out.reshape(1, S, D)
```

```python
import functools

import jax
import jax.numpy as jnp
import jax.experimental.pallas as pl
import jax.experimental.pallas.tpu as pltpu

f32 = jnp.float32
bf16 = jnp.bfloat16
u32 = jnp.uint32

S = 2048
D = 448
H = 16
DH = 256
M = 8
SEG = 32
NSEG = S // SEG
L = M + SEG
F = 1792
DP = 512
EPS = 1e-5
NEG = -1000000000.0
NB = S // 128

CH = 112
NCH = D // CH
X1 = 2
X2 = 2
NT = (((1,), (1,)), ((), ()))

SEM_Q, SEM_K, SEM_V = 0, 8, 16
SEM_O, SEM_M, SEM_G, SEM_U, SEM_D, SEM_MEM, SEM_C, SEM_R, SEM_X, SEM_OUT = range(24, 34)
NSEM = 34


def _rb(v):
    return v.astype(bf16).astype(f32)


def _ln(x):
    mu = jnp.mean(x, axis=-1, keepdims=True)
    xc = x - mu
    var = jnp.mean(xc * xc, axis=-1, keepdims=True)
    return xc * jax.lax.rsqrt(var + EPS)


def _dup_tail(v):
    return jnp.concatenate([v, v[:, 384:448]], axis=1)


def _kernel(xt_hbm, mem0_hbm, wq_hbm, wk_hbm, wv_hbm, wot_hbm, wr_hbm, wg_hbm, wu_hbm, wdt_hbm,
            c_hbm, wmod_hbm, out_hbm,
            rawq, rawk, rawv, q_s, wo_v, w_s, scr_a, scr_b, xt_v, x_rows, h_all, att, h2_all,
            o_rows, ot_v, wg_v, wu_v, wd_v, wmod_v, mem0_v, c_v, wr_v, sems):
    def chunk_copies(src, dst, k, i):
        r0 = pl.multiple_of(i * (CH * H), CH * H)
        return [pltpu.make_async_copy(src.at[pl.ds(r0, CH * H), pl.ds(j * 128, 128)],
                                      dst.at[j, pl.ds(r0, CH * H), :],
                                      sems.at[k + 2 * i + j]) for j in range(2)]

    cp_o = pltpu.make_async_copy(wot_hbm, wo_v, sems.at[SEM_O])
    cp_m = pltpu.make_async_copy(wmod_hbm, wmod_v, sems.at[SEM_M])
    cp_g = pltpu.make_async_copy(wg_hbm, wg_v, sems.at[SEM_G])
    cp_u = pltpu.make_async_copy(wu_hbm, wu_v, sems.at[SEM_U])
    cp_d = pltpu.make_async_copy(wdt_hbm, wd_v, sems.at[SEM_D])
    cp_small = [pltpu.make_async_copy(mem0_hbm, mem0_v, sems.at[SEM_MEM]),
                pltpu.make_async_copy(c_hbm, c_v, sems.at[SEM_C]),
                pltpu.make_async_copy(wr_hbm, wr_v, sems.at[SEM_R])]
    cp_x = []
    for b in range(NB):
        cols = pl.ds(b * 128, 128)
        cp_x.append(pltpu.make_async_copy(xt_hbm.at[:, cols], xt_v.at[b, pl.ds(0, D), :],
                                          sems.at[SEM_X]))
        cp_x.append(pltpu.make_async_copy(xt_hbm.at[pl.ds(384, 64), cols],
                                          xt_v.at[b, pl.ds(D, 64), :], sems.at[SEM_X]))

    def out_copy(b):
        cols = pl.ds(pl.multiple_of(b * 128, 128), 128)
        return pltpu.make_async_copy(ot_v.at[b, pl.ds(0, D), :], out_hbm.at[:, cols],
                                     sems.at[SEM_OUT])

    for i in range(NCH):
        for cp in chunk_copies(wq_hbm, rawq, SEM_Q, i):
            cp.start()
    for i in range(NCH):
        for cp in chunk_copies(wk_hbm, rawk, SEM_K, i):
            cp.start()
    cp_o.start()
    for i in range(NCH):
        for cp in chunk_copies(wv_hbm, rawv, SEM_V, i):
            cp.start()
    for cp in cp_small + cp_x + [cp_m]:
        cp.start()

    def head_pair(raw, i, p):
        r0 = pl.multiple_of(i * (CH * 8), CH * 8)
        r32 = raw.bitcast(u32)
        vs = [r32.at[j, pl.ds(r0, CH * 8), :][pl.ds(p, CH, stride=8), :] for j in range(2)]
        return [jnp.concatenate(
            [pltpu.unpack_elementwise(v, index=t, packed_dtype=bf16, unpacked_dtype=f32) for v in vs],
            axis=1) for t in range(2)]

    def store_pair(part, i, p, lo, hi):
        base = part * 56
        rows = pl.ds(pl.multiple_of(i * (CH // 2), 8), CH // 2)
        for t, a in enumerate((lo, hi)):
            for c in range(3):
                w_s[base + 8 + 16 * c + 2 * p + t, rows, :] = pltpu.bitcast(
                    a[:, c * 128:(c + 1) * 128].astype(bf16), u32)
        tl = jnp.concatenate([lo[:, 384:448], hi[:, 384:448]], axis=1)
        w_s[base + p, rows, :] = pltpu.bitcast(tl.astype(bf16), u32)

    def relayout_q(i, carry):
        for cp in chunk_copies(wq_hbm, rawq, SEM_Q, i):
            cp.wait()
        rows = pl.ds(pl.multiple_of(i * CH, 16), CH)
        for p in range(8):
            qs = head_pair(rawq, i, p)
            for t in range(2):
                q_s[2 * p + t, rows, :] = qs[t].astype(bf16)
        return carry

    jax.lax.fori_loop(0, NCH, relayout_q, 0)

    def fold(part, src_hbm, raw, sem0, rhs, scale):
        def body(i, carry):
            for cp in chunk_copies(src_hbm, raw, sem0, i):
                cp.wait()
            for p in range(8):
                ls = head_pair(raw, i, p)
                a = [jax.lax.dot_general(ls[t], rhs[2 * p + t], NT, preferred_element_type=f32)
                     for t in range(2)]
                if scale is not None:
                    a = [v * scale for v in a]
                store_pair(part, i, p, a[0], a[1])
            return carry
        jax.lax.fori_loop(0, NCH, body, 0)

    fold(0, wk_hbm, rawk, SEM_K, q_s, DH ** -0.5)
    cp_o.wait()
    fold(1, wv_hbm, rawv, SEM_V, wo_v, None)

    for cp in cp_small + cp_x + [cp_m]:
        cp.wait()
    for cp in (cp_g, cp_u, cp_d):
        cp.start()

    cc = c_v[...].astype(f32)
    sc = _rb(cc * jax.nn.sigmoid(cc))
    mod = jnp.dot(jnp.broadcast_to(sc, (8, D)), wmod_v[...], preferred_element_type=f32)[0:1]
    sa, ca, ga, sb, cb, gb = [mod[:, k * D:(k + 1) * D] for k in range(6)]
    ca1 = 1.0 + ca
    cb1 = 1.0 + cb
    wr = wr_v[...].astype(f32).reshape(1, D)

    def seg_rows(s):
        return pl.ds(pl.multiple_of(s * SEG, SEG), SEG)

    def blk_rows(b):
        return pl.ds(pl.multiple_of(b * 128, 128), 128)

    def xin(b, j):
        x_rows[blk_rows(b), j * 128:(j + 1) * 128] = xt_v[b, j * 128:(j + 1) * 128, :].astype(f32).T

    def xout(b, j):
        ot_v[b, j * 128:(j + 1) * 128, :] = o_rows[blk_rows(b), j * 128:(j + 1) * 128].T.astype(bf16)

    def ln1(s):
        x = x_rows[seg_rows(s), :D]
        h_all[seg_rows(s), :] = _dup_tail(_rb(_ln(x) * ca1 + sa))

    row_iota = jax.lax.broadcasted_iota(jnp.int32, (SEG, 1), 0)

    def finish(s, valid, best, bidx):
        x1 = x_rows[seg_rows(s), :D] + ga * att[:, :D]
        h2 = _ln(x1) * cb1 + sb
        h2_all[seg_rows(s), :] = h2
        o_rows[seg_rows(s), :] = _dup_tail(x1 + gb * h2)
        r = jnp.sum(h2 * wr, axis=-1, keepdims=True)
        better = r > best
        if valid is not True:
            better = jnp.logical_and(better, valid)
        return jnp.where(better, r, best), jnp.where(better, row_iota + s * SEG, bidx)

    qi = jax.lax.broadcasted_iota(jnp.int32, (L, 128), 0)
    ki = jax.lax.broadcasted_iota(jnp.int32, (L, 128), 1) // H

    def unit(lhs, row0, scr, part, u):
        n = lhs.shape[0]
        t0 = part * 56 + 2 * u
        w = jnp.concatenate([pltpu.bitcast(w_s[t0 + j], bf16) for j in range(2)], axis=1)
        y = jnp.dot(lhs, w, preferred_element_type=f32)
        if u >= 4:
            c, p = (u - 4) // 8, (u - 4) % 8
            pk = pltpu.pack_elementwise([y[:, :128], y[:, 128:]], packed_dtype=bf16)
            scr[c, pl.ds(row0 * 8 + p, n, stride=8), :] = pk
        else:
            lane = jax.lax.broadcasted_iota(jnp.int32, (n, 128), 1)
            for j in range(2):
                t = y[:, j * 128:(j + 1) * 128]
                pk = pltpu.pack_elementwise(
                    [jnp.where(lane < 64, t, 0.0), jnp.where(lane >= 64, t, 0.0)], packed_dtype=bf16)
                scr[3, pl.ds(row0 * 8 + 2 * u + j, n, stride=8), :] = pk

    X = X1 + X2
    for j in range(4):
        xin(0, j)
    ln1(0)
    att[...] = jnp.zeros(att.shape, f32)
    o_rows[blk_rows(0), :] = jnp.zeros((128, DP), f32)
    hx0 = h_all[seg_rows(0), :D]
    for u in range(X):
        unit(hx0, M, scr_a, 0, u)

    def step(s, sn, mem):
        h40 = jnp.concatenate([mem, h_all[seg_rows(s), :]], axis=0)
        h40a = h40[:, :D]
        k = 0
        for i, u in enumerate(range(X, 28)):
            unit(h40a, 0, scr_a, 0, u)
            if i % 3 == 2 and k < X:
                unit(h40a[:M], 0, scr_a, 0, k)
                k += 1
        st = []

        def s_tile(t):
            kst = jnp.concatenate(
                [pltpu.bitcast(scr_a[c, t * 64:(t + 1) * 64, :], bf16) for c in range(4)], axis=1)
            sc_ = jax.lax.dot_general(h40, kst, NT, preferred_element_type=f32)
            mask = jnp.logical_or(qi < M, qi >= ki + 8 * t)
            st.append(jnp.where(mask, sc_, NEG))

        for u in range(12):
            unit(h40a, 0, scr_b, 1, u)
            if u >= 2 and u % 2 == 0:
                s_tile(len(st))
        m = st[0]
        for t in range(1, 5):
            m = jnp.maximum(m, st[t])
        for sh in (16, 32, 64):
            m = jnp.maximum(m, pltpu.roll(m, sh, 1))
        e = [jnp.exp(st[t] - m) for t in range(5)]
        l = e[0] + e[1] + e[2] + e[3] + e[4]
        for sh in (16, 32, 64):
            l = l + pltpu.roll(l, sh, 1)
        r = 1.0 / l
        p = jnp.concatenate([_rb(v * r) for v in e], axis=1)

        def pz(c):
            return jnp.dot(p, pltpu.bitcast(scr_b[c], bf16), preferred_element_type=f32)

        for u in range(12, 24):
            unit(h40a, 0, scr_b, 1, u)
        tl = pz(3)
        o0 = pz(0)
        for u in range(24, 28):
            unit(h40a, 0, scr_b, 1, u)
        o1 = pz(1)
        hn = h_all[seg_rows(sn), :D]
        for u in range(X1):
            unit(hn, M, scr_a, 0, u)
        o2 = pz(2)
        for u in range(X1, X):
            unit(hn, M, scr_a, 0, u)
        tl = tl + pltpu.roll(tl, 64, 1)
        o = jnp.concatenate([o0, o1, o2, tl], axis=1)
        att[...] = o[M:]
        return _rb(o[:M])

    def block(b, carry):
        mem, best, bidx = carry

        @pl.when(b >= 2)
        def _():
            out_copy(b - 2).start()

        bn = jnp.minimum(b + 1, NB - 1)
        bp = jnp.maximum(b - 1, 0)
        for j in range(4):
            s = 4 * b + j
            if j == 0:
                best, bidx = finish(jnp.maximum(s - 1, 0), b > 0, best, bidx)
            else:
                best, bidx = finish(s - 1, True, best, bidx)
            sn = jnp.minimum(s + 1, NSEG - 1) if j == 3 else s + 1
            xin(bn, j)
            ln1(sn)
            xout(bp, j)
            mem = step(s, sn, mem)
        return mem, best, bidx

    mem0 = _dup_tail(mem0_v[...].astype(f32))
    best0 = jnp.full((SEG, 1), -jnp.inf, f32)
    bidx0 = jnp.zeros((SEG, 1), jnp.int32)
    _, best, bidx = jax.lax.fori_loop(0, NB, block, (mem0, best0, bidx0))
    out_copy(NB - 2).start()
    best, bidx = finish(NSEG - 1, True, best, bidx)

    rmax = jnp.max(best, axis=0, keepdims=True)
    idx = jnp.min(jnp.where(best == rmax, bidx, S))
    idx = jnp.clip(idx, 0, S - 1)
    for cp in (cp_g, cp_u, cp_d):
        cp.wait()
    xs = _rb(jnp.broadcast_to(h2_all[pl.ds(idx, 1), :], (8, D)))
    g = jnp.dot(xs, wg_v[...], preferred_element_type=f32)
    u = jnp.dot(xs, wu_v[...], preferred_element_type=f32)
    a = _rb(g * jax.nn.sigmoid(g) * u)
    y = jax.lax.dot_general(a, wd_v[...], NT, preferred_element_type=f32)[0:1]
    y = y * jax.nn.sigmoid(rmax)
    o_rows[pl.ds(idx, 1), :] = o_rows[pl.ds(idx, 1), :] + _dup_tail(gb * y)
    for j in range(4):
        xout(NB - 1, j)
    for b in range(NB - 1):
        out_copy(b).wait()
    out_copy(NB - 1).start()
    bsel = jnp.minimum(idx // 128, NB - 2)
    for j in range(4):
        xout(bsel, j)
    out_copy(bsel).start()
    out_copy(NB - 1).wait()
    out_copy(bsel).wait()


@functools.partial(jax.jit, static_argnames=("A_seg_len",))
def pallas_adaLN_cond__memory_aug_recurrent_mem_tr__moe_arch_mod__prompt_kernel(
    A_x, A_mem0, A_Wq, A_Wk, A_Wv, A_Wo, A_seg_len, B_x, B_w_r, B_w_gate, B_w_up, B_w_down,
    c, w_mod,
):
    del B_x
    assert int(A_seg_len) == SEG and A_x.shape == (1, S, D)
    hbm = pl.BlockSpec(memory_space=pltpu.HBM)
    out_t = pl.pallas_call(
        _kernel,
        out_shape=jax.ShapeDtypeStruct((D, S), A_x.dtype),
        in_specs=[hbm] * 12,
        out_specs=hbm,
        scratch_shapes=[
            pltpu.VMEM((2, D * H, 128), bf16),
            pltpu.VMEM((2, D * H, 128), bf16),
            pltpu.VMEM((2, D * H, 128), bf16),
            pltpu.VMEM((H, D, DH), bf16),
            pltpu.VMEM((H, D, DH), bf16),
            pltpu.VMEM((112, D // 2, 128), u32),
            pltpu.VMEM((4, L * 8, 128), u32),
            pltpu.VMEM((4, L * 8, 128), u32),
            pltpu.VMEM((NB, DP, 128), bf16),
            pltpu.VMEM((S, DP), f32),
            pltpu.VMEM((S, DP), f32),
            pltpu.VMEM((SEG, DP), f32),
            pltpu.VMEM((S, D), f32),
            pltpu.VMEM((S, DP), f32),
            pltpu.VMEM((NB, DP, 128), bf16),
            pltpu.VMEM((D, F), bf16),
            pltpu.VMEM((D, F), bf16),
            pltpu.VMEM((D, F), bf16),
            pltpu.VMEM((D, 6 * D), bf16),
            pltpu.VMEM((M, D), bf16),
            pltpu.VMEM((1, D), bf16),
            pltpu.VMEM((D,), bf16),
            pltpu.SemaphoreType.DMA((NSEM,)),
        ],
        compiler_params=pltpu.CompilerParams(vmem_limit_bytes=100 * 1024 * 1024),
    )(
        A_x.reshape(S, D).T, A_mem0.reshape(M, D),
        A_Wq.reshape(D * H, DH), A_Wk.reshape(D * H, DH), A_Wv.reshape(D * H, DH),
        jnp.swapaxes(A_Wo, 1, 2), B_w_r, B_w_gate, B_w_up, B_w_down.T, c, w_mod,
    )
    return out_t.T.reshape(1, S, D)
```

```python
import functools
import re

import jax
import jax.numpy as jnp
import jax.experimental.pallas as pl
import jax.experimental.pallas.tpu as pltpu

f32 = jnp.float32
bf16 = jnp.bfloat16
u32 = jnp.uint32

S = 2048
D = 448
H = 16
DH = 256
M = 8
SEG = 32
NSEG = S // SEG
L = M + SEG
F = 1792
DP = 512
EPS = 1e-5
NEG = -1000000000.0
NB = S // 128

SCHEDULE = (
    "q0 a7 a4 q1 a5 q2 q3 a6 a9 a2 a1 a0 a8 r0 a10 r1 a3 a11 r2 a12 r3 a13 r4 a14 s30 a15 s31 "
    "a16 s32 a17 s33 a18 s34 a19 s00 a20 s01 a21 s02 a22 s03 a23 s04 a24 s10 a25 s11 a26 a27 "
    "s14 s12 b0 b1 b2 s13 b3 s20 s21 b4 s22 s23 b5 s24 sm b6 b7 b8 b10 b11 b12 b9 b13 b14 b16 "
    "b17 b18 b19 B15 b20 b21 t0 t4 t3 t7 t5 t6 t1 pz3 t2 pz0 pz1 b22 b23 tb1 tb3 b24 tb0 b25 "
    "b27 b26 tb2 ea6 ea18 ea5 ea4 pz2 ea11 ea9 ea10 ea7 "
)
EARLY = [(op[1], int(op[2:])) for op in SCHEDULE.split() if op[0] == "e"]
BPI = 2
RED_LEVELS = [(16, 32, 48), (64,)]
NT = (((1,), (1,)), ((), ()))

SEM_Q, SEM_L = 0, 7
SEM_O, SEM_PRE, SEM_LATE, SEM_OUT = range(15, 19)
NSEM = 19


def _rb(v):
    return v.astype(bf16).astype(f32)


def _bits(v, dtype):
    return jax.lax.bitcast_convert_type(v, dtype)


def _pack2(lo, hi):
    return (_bits(_rb(lo), u32) >> 16) | _bits(_rb(hi), u32)


def _unpack2(v, t):
    return _bits(v << 16 if t == 0 else v & jnp.uint32(0xFFFF0000), f32)


def _split(v):
    return [v[:8], v[8:]]


def _add_split(parts, v):
    return jnp.concatenate([parts[0] + v[:8], parts[1] + v[8:]], axis=0)


def _ln(x):
    mu = jnp.mean(x, axis=-1, keepdims=True)
    xc = x - mu
    var = jnp.mean(xc * xc, axis=-1, keepdims=True)
    return xc * jax.lax.rsqrt(var + EPS)


def _dup_tail(v):
    return jnp.concatenate([v, v[:, 384:448]], axis=1)


def _kernel(xt_hbm, mem0_hbm, wq_hbm, wk_hbm, wv_hbm, wot_hbm, wr_hbm, wg_hbm, wu_hbm, wdt_hbm,
            c_hbm, wmod_hbm, out_hbm,
            rawq, raw, rhs, w_s, w_q, w_bt, bd, part_buf, scr_a, scr_b, xt_v, x_rows, hbuf, att,
            h2_all, o_rows, ot_v, r_all, wg_v, wu_v, wd_v, wmod_v, mem0_v, c_v, wr_v, sems):
    def row_copies(src, dst, sem, d0, n):
        rows = pl.ds(pl.multiple_of(d0 * H, 1024), n * H)
        return [pltpu.make_async_copy(src.at[rows, pl.ds(j * 128, 128)], dst.at[j, rows, :],
                                      sems.at[sem]) for j in range(2)]

    def q_copies(i):
        return row_copies(wq_hbm, rawq, SEM_Q + i, i * 64, 64)

    def lhs_copies(src, part, i):
        if i is None:
            return row_copies(src, raw.at[part], SEM_L + 4 * part + 3, 384, 64)
        return row_copies(src, raw.at[part], SEM_L + 4 * part + i, i * 128, 128)

    cp_o = pltpu.make_async_copy(wot_hbm, rhs.at[1], sems.at[SEM_O])
    cp_m = pltpu.make_async_copy(wmod_hbm, wmod_v, sems.at[SEM_PRE])
    cp_g = pltpu.make_async_copy(wg_hbm, wg_v, sems.at[SEM_LATE])
    cp_u = pltpu.make_async_copy(wu_hbm, wu_v, sems.at[SEM_LATE])
    cp_d = pltpu.make_async_copy(wdt_hbm, wd_v, sems.at[SEM_LATE])
    cp_small = [pltpu.make_async_copy(mem0_hbm, mem0_v, sems.at[SEM_PRE]),
                pltpu.make_async_copy(c_hbm, c_v, sems.at[SEM_PRE]),
                pltpu.make_async_copy(wr_hbm, wr_v, sems.at[SEM_PRE])]

    def x_copies(b):
        cols = pl.ds(b * 128, 128)
        sem = sems.at[SEM_PRE if b <= BPI else SEM_LATE]
        return [pltpu.make_async_copy(xt_hbm.at[:, cols], xt_v.at[b, pl.ds(0, D), :], sem),
                pltpu.make_async_copy(xt_hbm.at[pl.ds(384, 64), cols],
                                      xt_v.at[b, pl.ds(D, 64), :], sem)]

    def out_copy(b, slot=None):
        cols = pl.ds(pl.multiple_of(b * 128, 128), 128)
        return pltpu.make_async_copy(ot_v.at[b if slot is None else slot, pl.ds(0, D), :],
                                     out_hbm.at[:, cols], sems.at[SEM_OUT])

    for i in range(7):
        for cp in q_copies(i):
            cp.start()
    for i in (None, 0, 1, 2):
        for cp in lhs_copies(wk_hbm, 0, i):
            cp.start()
    cp_o.start()
    for i in (None, 0, 1, 2):
        for cp in lhs_copies(wv_hbm, 1, i):
            cp.start()
    cp_pre = cp_small + sum([x_copies(b) for b in range(BPI + 1)], []) + [cp_m]
    cp_late = sum([x_copies(b) for b in range(BPI + 1, NB)], []) + [cp_g, cp_u, cp_d]
    for cp in cp_pre + cp_late:
        cp.start()

    def head_pair(ref, d0, n, p):
        rows = pl.ds(pl.multiple_of(d0 * 8, 512), n * 8)
        vs = [ref.at[j, rows, :][pl.ds(p, n, stride=8), :] for j in range(2)]
        return [jnp.concatenate(
            [_unpack2(v, t) for v in vs],
            axis=1) for t in range(2)]

    def to_u32(v):
        return pltpu.bitcast(v.astype(bf16), u32)

    def relayout_q(i, carry):
        for cp in q_copies(i):
            cp.wait()
        rows = pl.ds(pl.multiple_of(i * 64, 64), 64)
        for p in range(8):
            qs = head_pair(rawq.bitcast(u32), i * 64, 64, p)
            for t in range(2):
                rhs[0, 2 * p + t, rows, :] = (qs[t] * (DH ** -0.5)).astype(bf16)
        return carry

    jax.lax.fori_loop(0, 7, relayout_q, 0)

    def build_wq(p):
        def tail_rows(t):
            return pltpu.bitcast(w_s[t, 192:224, :], bf16).astype(f32)
        for c in range(3):
            blk = jnp.concatenate([tail_rows(8 + 16 * c + 2 * p + t) for t in range(2)], axis=0)
            w_q[p, c * 64:(c + 1) * 64, :] = pltpu.bitcast(blk.T.astype(bf16), u32)
        r = tail_rows(p)
        blk = jnp.concatenate([r, pltpu.roll(r, 64, 1)], axis=0)
        w_q[p, 192:224, :] = pltpu.bitcast(blk.T[:64].astype(bf16), u32)

    def fold(part, carry):
        base = part * 56
        src = raw.bitcast(u32).at[part]

        @pl.when(part == 1)
        def _():
            cp_o.wait()

        for cp in lhs_copies(wk_hbm, part, None):
            cp.wait()
        for p in range(8):
            ls = head_pair(src, 384, 64, p)
            a = [jax.lax.dot_general(ls[t], rhs[part, 2 * p + t], NT, preferred_element_type=f32)
                 for t in range(2)]
            for t in range(2):
                for c in range(3):
                    w_s[base + 8 + 16 * c + 2 * p + t, 192:224, :] = to_u32(
                        a[t][:, c * 128:(c + 1) * 128])
            w_s[base + p, 192:224, :] = to_u32(
                jnp.concatenate([a[0][:, 384:], a[1][:, 384:]], axis=1))

        def body(i, carry):
            for cp in lhs_copies(wk_hbm, part, i):
                cp.wait()
            p0 = jnp.minimum(2 * (3 * part + i), 6)
            build_wq(p0)
            build_wq(p0 + 1)
            rows = pl.ds(pl.multiple_of(i * 64, 64), 64)
            for p in range(8):
                ls = head_pair(src, i * 128, 128, p)
                tt = [jax.lax.dot_general(rhs[part, 2 * p + t, 384:, :], ls[t].astype(bf16), NT,
                                          preferred_element_type=f32) for t in range(2)]
                w_s[base + p, rows, :] = to_u32(jnp.concatenate(tt, axis=0).T)
                for t in range(2):
                    h = 2 * p + t
                    a = jax.lax.dot_general(ls[t], rhs[part, h, :384, :], NT,
                                            preferred_element_type=f32)
                    for c in range(3):
                        w_s[base + 8 + 16 * c + h, rows, :] = to_u32(a[:, c * 128:(c + 1) * 128])
            return carry

        return jax.lax.fori_loop(0, 3, body, carry)

    jax.lax.fori_loop(0, 2, fold, 0)

    for cp in cp_pre:
        cp.wait()

    cc = c_v[...].astype(f32)
    sc = _rb(cc * jax.nn.sigmoid(cc))
    mod = jnp.dot(jnp.broadcast_to(sc, (8, D)), wmod_v[...], preferred_element_type=f32)[0:1]
    sa, ca, ga, sb, cb, gb = [mod[:, k * D:(k + 1) * D] for k in range(6)]
    ca1 = 1.0 + ca
    cb1 = 1.0 + cb
    wr = wr_v[...].astype(f32).reshape(1, D)

    def seg_rows(s):
        return pl.ds(pl.multiple_of(s * SEG, SEG), SEG)

    def blk_rows(b):
        return pl.ds(pl.multiple_of(b * 128, 128), 128)

    def xin(b, j):
        x_rows[blk_rows(b), j * 128:(j + 1) * 128] = xt_v[b, j * 128:(j + 1) * 128, :].astype(f32).T

    def fold_rows(v):
        acc = None
        for i in range(v.shape[0] // 8):
            for j in range(v.shape[1] // 128):
                t = v[i * 8:(i + 1) * 8, j * 128:(j + 1) * 128]
                acc = t if acc is None else jnp.maximum(acc, t)
        return acc

    def xout(b, j, slot=None, add=None):
        t = o_rows[blk_rows(b), j * 128:(j + 1) * 128]
        if add is not None:
            t = t + add[:, j * 128:(j + 1) * 128]
        t = t.T
        ot_v[b if slot is None else slot, j * 128:(j + 1) * 128, :] = t.astype(bf16)
        if j == 3 and slot is None:
            r_all[pl.ds(b, 1), :] = t[64:65, :]
        return fold_rows(t)

    def ln1(s, slot):
        x = x_rows[seg_rows(s), :D]
        h = _dup_tail(_rb(_ln(x) * ca1 + sa))
        hbuf[slot] = h
        return fold_rows(h)

    def finish(s, slot):
        x1 = x_rows[seg_rows(s), :D] + ga * att[slot, :, :D]
        h2 = _ln(x1) * cb1 + sb
        h2_all[seg_rows(s), :] = h2
        r = jnp.sum(h2 * wr, axis=-1, keepdims=True)
        o = jnp.concatenate([x1 + gb * h2, jnp.broadcast_to(r, (SEG, 64))], axis=1)
        o_rows[seg_rows(s), :] = o
        return fold_rows(o), r

    sub8 = jax.lax.broadcasted_iota(jnp.int32, (8, 128), 0)
    gran8 = jax.lax.broadcasted_iota(jnp.int32, (8, 128), 1) // H

    def gran_t(x):
        for b in (4, 2, 1):
            sbit = (sub8 & b) != 0
            gbit = (gran8 & b) != 0
            if b == 4:
                v = pltpu.roll(pltpu.roll(x, 64, 1), 4, 0)
            else:
                z = jnp.where(sbit, pltpu.roll(x, 16 * b, 1), pltpu.roll(x, 128 - 16 * b, 1))
                v = jnp.where(sbit, pltpu.roll(z, b, 0), pltpu.roll(z, 8 - b, 0))
            x = jnp.where(sbit != gbit, v, x)
        return x

    def lane_reduce(op, x):
        for level in RED_LEVELS:
            vs = [x] + [pltpu.roll(x, sh, 1) for sh in level]
            while len(vs) > 1:
                vs = [op(vs[i], vs[i + 1]) for i in range(0, len(vs), 2)]
            x = vs[0]
        return x

    lane32 = jax.lax.broadcasted_iota(jnp.int32, (32, 128), 1)
    for p in range(8):
        v = w_s[56 + p, 192:224, :]
        w_bt[p, :32, :] = jnp.where(lane32 < 64, v, jnp.uint32(0))
        w_bt[p, 32:, :] = jnp.where(lane32 >= 64, v, jnp.uint32(0))
    bd[...] = jnp.zeros(bd.shape, u32)
    r_all[...] = jnp.zeros(r_all.shape, f32)
    lane8 = jax.lax.broadcasted_iota(jnp.int32, (8, 128), 1)
    lane40 = jax.lax.broadcasted_iota(jnp.int32, (L, 128), 1)
    slot8 = (lane8 % H) // 2
    for j in range(4):
        xin(0, j)
    ln1(0, 0)
    att[3] = jnp.zeros((SEG, DP), f32)
    o_rows[blk_rows(0), :] = jnp.zeros((128, DP), f32)

    def _pack_halves(v):
        w = _bits(_rb(v), u32)
        return jnp.where(lane40 < 64, w >> 16, w)

    def groups_for_key_tile(t):
        return [0] + list(range(max(t, 1), 5))

    def key_tiles(g):
        return range(5) if g == 0 else range(g + 1)

    class Step:
        def __init__(self, j, never, spill=False):
            self.j, self.never, self.spill = j, never, spill
            self.mem = {}
            self.hc_ = {}
            self.part = {}
            self.sc = {}
            self.tp = {}
            self.oc = {}
            self.dep = None
            self.out = {}

        def hc(self, c):
            if c not in self.hc_:
                self.hc_[c] = jnp.concatenate(
                    [self.mem[c], hbuf[self.j, :, c * 128:(c + 1) * 128]], axis=0)
            return self.hc_[c]

        def mm(self, kind, u, cs, tie=False):
            ref, t0 = {"a": (w_s, 0), "q": (w_q, 0), "b": (w_s, 56)}[kind]
            ls, ws = [], []
            for c in cs:
                h = self.hc(c)
                if tie and c == cs[0]:
                    h = jnp.concatenate([jnp.where(self.never, self.dep, h[:8]), h[8:]], axis=0)
                ls.append(h if c < 3 else h[:, :64])
                r0, r1 = c * 64, (c * 64 + 64 if c < 3 else 224)
                ws.append(jnp.concatenate(
                    [pltpu.bitcast(ref[t0 + 2 * u + i, r0:r1, :], bf16) for i in range(2)], axis=1))
            return jnp.dot(jnp.concatenate(ls, axis=1), jnp.concatenate(ws, axis=0),
                           preferred_element_type=f32)

        def early(self, kind, u):
            y = self.mm(kind, u, (0, 1, 3) if kind == "q" else (0, 1))
            if self.spill:
                part_buf[EARLY.index((kind, u))] = y
            else:
                self.part[(kind, u)] = _split(y)

        def unit(self, kind, u, tie=False):
            if (kind, u) in self.part:
                y = _add_split(self.part[(kind, u)], self.mm(kind, u, (2,)))
            else:
                y = self.mm(kind, u, (0, 1, 2, 3) if kind == "q" else (0, 1, 2), tie)
            scr = (scr_b if kind == "b" else scr_a).at[self.j]
            ys = [y[:, :128], y[:, 128:]]
            if u < 4:
                for i in range(2):
                    pk = _pack_halves(ys[i])
                    scr[4 if kind == "q" else 3, pl.ds(2 * u + i, L, stride=8), :] = pk
            else:
                pk = _pack2(*ys)
                scr[(u - 4) // 8, pl.ds((u - 4) % 8, L, stride=8), :] = pk

        def add_sc(self, k, v):
            self.sc[k] = v + self.sc[k] if k in self.sc else v

        def s_tile(self, c, t):
            gs = groups_for_key_tile(t)
            kst = pltpu.bitcast(scr_a[self.j, c, t * 64:(t + 1) * 64, :], bf16)
            lhs = jnp.concatenate([self.hc(c)[8 * g:8 * (g + 1)] for g in gs], axis=0)
            v = jax.lax.dot_general(lhs, kst, NT, preferred_element_type=f32)
            for i, g in enumerate(gs):
                self.add_sc((g, t), v[8 * i:8 * (i + 1)])

        def s2_tile(self, g):
            nk = len(key_tiles(g))
            qst = pltpu.bitcast(scr_a[self.j, 4, g * 64:(g + 1) * 64, :], bf16)
            v = jax.lax.dot_general(self.hc(3)[:8 * nk], qst, NT, preferred_element_type=f32)
            for t in range(nk):
                self.add_sc((g, t), gran_t(v[8 * t:8 * (t + 1)]))

        def softmax(self):
            sc, pr = self.sc, {}
            for g in range(5):
                ts = key_tiles(g)
                if g > 0:
                    sc[(g, g)] = jnp.where(sub8 >= gran8, sc[(g, g)], NEG)
                m = functools.reduce(jnp.maximum, [sc[(g, t)] for t in ts])
                m = lane_reduce(jnp.maximum, m)
                e = [jnp.exp(sc[(g, t)] - m) for t in ts]
                l = lane_reduce(jnp.add, functools.reduce(lambda a, b: a + b, e))
                r = 1.0 / l
                for t in ts:
                    pr[(g, t)] = _rb(e[t] * r)
            self.p01 = jnp.concatenate(
                [jnp.concatenate([pr[(g, 0)], pr[(g, 1)]], axis=1) for g in range(5)], axis=0)
            self.pt = {t: jnp.concatenate([pr[(g, t)] for g in groups_for_key_tile(t)], axis=0)
                       for t in (2, 3, 4)}
            self.rolled = {k: (v if k[1] == 0 else pltpu.roll(v, 2 * k[1], 1))
                           for k, v in pr.items()}
            ht = self.hc(3)
            pk = _pack_halves(ht)
            for g in range(5):
                bd[self.j, pl.ds(g, 8, stride=8), :] = pk[8 * g:8 * (g + 1)]
                bd[self.j, pl.ds(64 + g, 8, stride=8), :] = pk[8 * g:8 * (g + 1)]

        def t_pair(self, p):
            rows = []
            for g in range(5):
                ts = key_tiles(g)
                acc = self.rolled[(g, 0)]
                if len(ts) < 5:
                    acc = jnp.where(slot8 == p, acc, 0.0)
                for t in ts[1:]:
                    acc = jnp.where(slot8 == (p + t) % 8, self.rolled[(g, t)], acc)
                rows.append(acc)
            self.tp[p] = _rb(jnp.dot(jnp.concatenate(rows, axis=0),
                                     pltpu.bitcast(bd[self.j, 64 - p:128 - p, :], bf16),
                                     preferred_element_type=f32))

        def add_o(self, c, v):
            if c not in self.oc:
                self.oc[c] = _split(v)
                return
            o = _add_split(self.oc[c], v)
            if c == 3:
                o = o + pltpu.roll(o, 64, 1)
            att[self.j, :, c * 128:(c + 1) * 128] = o[M:]
            self.out[c] = _rb(o[:M])

        def tb(self, c):
            if c == 3:
                ws = [w_bt[p] for p in range(8)]
            else:
                ws = [w_s[56 + 8 + 16 * c + h, 192:224, :] for h in range(H)]
            tc = jnp.concatenate([self.tp[p] for p in range(8)], axis=1)
            self.add_o(c, jnp.dot(tc, pltpu.bitcast(jnp.concatenate(ws, axis=0), bf16),
                                  preferred_element_type=f32))

        def pz(self, c):
            z = scr_b.at[self.j, c]
            v = jnp.dot(self.p01, pltpu.bitcast(z[:128, :], bf16), preferred_element_type=f32)
            og = [v[8 * g:8 * (g + 1)] for g in range(5)]
            for t in (2, 3, 4):
                v = jnp.dot(self.pt[t], pltpu.bitcast(z[t * 64:(t + 1) * 64, :], bf16),
                            preferred_element_type=f32)
                for i, g in enumerate(groups_for_key_tile(t)):
                    og[g] = og[g] + v[8 * i:8 * (i + 1)]
            self.add_o(c, jnp.concatenate(og, axis=0))

        def run(self, nxt):
            nxt.mem = self.out
            for op in SCHEDULE.split():
                k, a = re.match(r"([a-zA-Z]+)(\d*)", op).groups()
                if k in ("q", "a", "b"):
                    self.unit(k, int(a))
                elif k == "B":
                    self.unit("b", int(a), tie=True)
                elif k == "r":
                    self.s2_tile(int(a))
                elif k == "s":
                    self.s_tile(int(a[0]), int(a[1]))
                elif k == "sm":
                    self.softmax()
                elif k == "t":
                    self.t_pair(int(a))
                elif k == "tb":
                    self.tb(int(a))
                elif k == "pz":
                    self.pz(int(a))
                elif k in ("eq", "ea", "eb"):
                    nxt.early(k[1], int(a))
                else:
                    raise ValueError(op)

    def block(it, mem):
        b0 = it * BPI
        for k in range(BPI):
            @pl.when(b0 - 2 - k >= 0)
            def _():
                out_copy(b0 - 2 - k).start()

        @pl.when(it == 1)
        def _():
            for cp in cp_late:
                cp.wait()

        never = it < 0
        n = 4 * BPI
        steps = [Step(j % 4, never) for j in range(n)] + [Step(0, never, spill=True)]
        steps[0].mem = {c: mem[:, c * 128:(c + 1) * 128] for c in range(4)}
        steps[0].part = {k: _split(part_buf[i]) for i, k in enumerate(EARLY)}
        for i in range(n):
            b, j = b0 + i // 4, i % 4
            s = 4 * b + j
            bn = jnp.minimum(b + 1, NB - 1) if i // 4 == BPI - 1 else b + 1
            bp = jnp.maximum(b - 1, 0) if i // 4 == 0 else b - 1
            sp = jnp.maximum(s - 1, 0) if i == 0 else s - 1
            sn = jnp.minimum(s + 1, NSEG - 1) if i == n - 1 else s + 1
            d1, _ = finish(sp, (j + 3) % 4)
            xin(bn, j)
            d3 = ln1(sn, (j + 1) % 4)
            d2 = xout(bp, j)
            steps[i].dep = jnp.maximum(jnp.maximum(d1, d2), d3)
            steps[i].run(steps[i + 1])
        return jnp.concatenate([steps[n - 1].out[c] for c in range(4)], axis=1)

    mem0 = _dup_tail(mem0_v[...].astype(f32))
    first = Step(0, None, spill=True)
    first.mem = {c: mem0[:, c * 128:(c + 1) * 128] for c in range(4)}
    for k in EARLY:
        first.early(*k)
    jax.lax.fori_loop(0, NB // BPI, block, mem0)
    for k in range(BPI):
        out_copy(NB - 2 - k).start()

    def argmax(v, tok):
        m = jnp.max(jnp.max(v, axis=0, keepdims=True), axis=1, keepdims=True)
        i = jnp.where(v == m, tok, S)
        return m, jnp.min(jnp.min(i, axis=0, keepdims=True), axis=1, keepdims=True)

    def iota(n, axis):
        return jax.lax.broadcasted_iota(jnp.int32, (n, 128), axis)

    n3 = 3 * SEG
    v1 = jnp.concatenate([
        jnp.where(iota(NB, 0) < NB - 1, r_all[...], -jnp.inf),
        jnp.where(iota(n3, 1) >= 64, o_rows[S - 128:S - SEG, 384:], -jnp.inf)], axis=0)
    t1 = jnp.concatenate([iota(NB, 0) * 128 + iota(NB, 1), iota(n3, 0) + (S - 128)], axis=0)
    m1, i1 = argmax(v1, t1)
    _, r_last = finish(NSEG - 1, 3)
    m2, i2 = argmax(r_last, jax.lax.broadcasted_iota(jnp.int32, (SEG, 1), 0) + (S - SEG))
    rmax = jnp.maximum(m1, m2)
    idx = jnp.clip(jnp.min(jnp.where(m2 > m1, i2, i1)), 0, S - 1)
    for j in range(4):
        xout(NB - 1, j, slot=NB - 1)
    out_copy(NB - 1).start()
    xs = _rb(jnp.broadcast_to(h2_all[pl.ds(idx, 1), :], (8, D)))
    g = jnp.dot(xs, wg_v[...], preferred_element_type=f32)
    u = jnp.dot(xs, wu_v[...], preferred_element_type=f32)
    a = _rb(g * jax.nn.sigmoid(g) * u)
    y = jax.lax.dot_general(a, wd_v[...], NT, preferred_element_type=f32)[0:1]
    y = y * jax.nn.sigmoid(rmax)
    bsel = jnp.clip(idx // 128, 0, NB - 1)
    hit = jax.lax.broadcasted_iota(jnp.int32, (128, 1), 0) == idx % 128
    upd = jnp.where(hit, jnp.concatenate([gb * y, jnp.zeros((1, 64), f32)], axis=1), 0.0)
    for j in range(4):
        xout(bsel, j, slot=NB, add=upd)
    for b in range(NB):
        out_copy(b).wait()
    out_copy(bsel, slot=NB).start()
    out_copy(bsel, slot=NB).wait()


@jax.jit
def pallas_adaLN_cond__memory_aug_recurrent_mem_tr__moe_arch_mod__prompt_kernel(
    A_x, A_mem0, A_Wq, A_Wk, A_Wv, A_Wo, A_seg_len, B_x, B_w_r, B_w_gate, B_w_up, B_w_down,
    c, w_mod,
):
    del B_x, A_seg_len
    assert A_x.shape == (1, S, D)
    hbm = pl.BlockSpec(memory_space=pltpu.HBM)
    out_t = pl.pallas_call(
        _kernel,
        out_shape=jax.ShapeDtypeStruct((D, S), A_x.dtype),
        in_specs=[hbm] * 12,
        out_specs=hbm,
        scratch_shapes=[
            pltpu.VMEM((2, D * H, 128), bf16),
            pltpu.VMEM((2, 2, D * H, 128), bf16),
            pltpu.VMEM((2, H, D, DH), bf16),
            pltpu.VMEM((112, D // 2, 128), u32),
            pltpu.VMEM((8, D // 2, 128), u32),
            pltpu.VMEM((8, 64, 128), u32),
            pltpu.VMEM((4, 128, 128), u32),
            pltpu.VMEM((len(EARLY), L, 256), f32),
            pltpu.VMEM((4, 5, L * 8, 128), u32),
            pltpu.VMEM((4, 4, L * 8, 128), u32),
            pltpu.VMEM((NB, DP, 128), bf16),
            pltpu.VMEM((S, DP), f32),
            pltpu.VMEM((4, SEG, DP), f32),
            pltpu.VMEM((4, SEG, DP), f32),
            pltpu.VMEM((S, D), f32),
            pltpu.VMEM((S, DP), f32),
            pltpu.VMEM((NB + 1, DP, 128), bf16),
            pltpu.VMEM((NB, 128), f32),
            pltpu.VMEM((D, F), bf16),
            pltpu.VMEM((D, F), bf16),
            pltpu.VMEM((D, F), bf16),
            pltpu.VMEM((D, 6 * D), bf16),
            pltpu.VMEM((M, D), bf16),
            pltpu.VMEM((1, D), bf16),
            pltpu.VMEM((D,), bf16),
            pltpu.SemaphoreType.DMA((NSEM,)),
        ],
        compiler_params=pltpu.CompilerParams(vmem_limit_bytes=100 * 1024 * 1024),
    )(
        A_x.reshape(S, D).T, A_mem0.reshape(M, D),
        A_Wq.reshape(D * H, DH), A_Wk.reshape(D * H, DH), A_Wv.reshape(D * H, DH),
        jnp.swapaxes(A_Wo, 1, 2), B_w_r, B_w_gate, B_w_up, B_w_down.T, c, w_mod,
    )
    return out_t.T.reshape(1, S, D)
```
